```python
import os as _os
_os.environ.setdefault("JAX_PLATFORMS", "cpu")
import jax
import jax.numpy as jnp

def _softmax(x, axis=-1):
    return jax.nn.softmax(x, axis=axis)
def _gelu(x):
    return jax.nn.gelu(x, approximate=True)
def _silu(x):
    return jax.nn.silu(x)
def _sigmoid(x):
    return jax.nn.sigmoid(x)
def _layernorm(x, axis=-1, eps=1e-5):
    m = jnp.mean(x, axis=axis, keepdims=True)
    v = jnp.var(x, axis=axis, keepdims=True)
    return (x - m) / jnp.sqrt(v + eps)
def _scatter_add(tgt, idx, src, axis=0):
    return tgt.at[idx].add(src)
def _segment_sum(src, seg, n):
    return jax.ops.segment_sum(src, seg, n)
class _Rng:
    def __init__(self, key):
        self._k = key
    def _next(self):
        self._k, sub = jax.random.split(self._k)
        return sub
    def normal(self, shape):
        return jax.random.normal(self._next(), shape, dtype=jnp.bfloat16)
    def randint(self, lo, hi, shape):
        return jax.random.randint(self._next(), shape, lo, hi, dtype=jnp.int32)
    def uniform(self, shape, lo=0.0, hi=1.0):
        return jax.random.uniform(self._next(), shape, jnp.bfloat16, lo, hi)
    def permutation(self, n):
        return jax.random.permutation(self._next(), n)


kernel_name = 'recurrent_scan__grouped_kv_mqa__mixer_s_mlp__prompt'

def setup_inputs():
    _rng = _Rng(jax.random.key(int.from_bytes(__import__("os").urandom(4), "little")))
    _w = (lambda a: (lambda t: t.astype(jnp.bfloat16) if jnp.issubdtype(t.dtype, jnp.floating) else t)(jnp.asarray(a)))
    def _A_setup():
        B, S, D, H = 1, 2048, 512, 32
        Dh = D // H
        return {
            "x": _w((lambda *s: _rng.normal(s) * 0.05)(B, S, D)),
            "wq": _w((lambda *s: _rng.normal(s) * 0.05)(D, H * Dh)),
            "wk": _w((lambda *s: _rng.normal(s) * 0.05)(D, Dh)),
            "wv": _w((lambda *s: _rng.normal(s) * 0.05)(D, Dh)),
            "wo": _w((lambda *s: _rng.normal(s) * 0.05)(H * Dh, D)),
        }
    _A_in = _A_setup()

    def _B_setup():
        B, S, D, F = 1, 2048, 512, 1792
        return {
            "x":  _w((lambda *s: _rng.normal(s) * 0.05)(B, S, D)),
            "w1": _w((lambda *s: _rng.normal(s) * 0.8)(D, D) * (D ** -0.5)),
            "w2": _w((lambda *s: _rng.normal(s) * 0.8)(D, D) * (D ** -0.5)),
            "w3": _w((lambda *s: _rng.normal(s) * 0.8)(D, F) * (D ** -0.5)),
            "w4": _w((lambda *s: _rng.normal(s) * 0.8)(F, D) * (F ** -0.5)),
        }
    _B_in = _B_setup()

    return {
        "A_x": _A_in["x"],
        "A_wq": _A_in["wq"],
        "A_wk": _A_in["wk"],
        "A_wv": _A_in["wv"],
        "A_wo": _A_in["wo"],
        "B_x": _B_in["x"],
        "B_w1": _B_in["w1"],
        "B_w2": _B_in["w2"],
        "B_w3": _B_in["w3"],
        "B_w4": _B_in["w4"],
    }

def reference(A_x, A_wq, A_wk, A_wv, A_wo, B_x, B_w1, B_w2, B_w3, B_w4):
    def _A_ref(x, wq, wk, wv, wo):
        B, S, D = x.shape
        H = 32
        Dh = D // H
        q = (lambda x, *d: x.transpose(*d))((x @ wq).reshape(B, S, H, Dh), 0, 2, 1, 3)
        k = x @ wk
        v = x @ wv
        scores = jnp.einsum("bhqd,bkd->bhqk", q, k) * (Dh ** -0.5)
        p = _softmax(scores, axis=-1)
        o = jnp.einsum("bhqk,bkd->bhqd", p, v)
        return (lambda x, *d: x.transpose(*d))(o, 0, 2, 1, 3).reshape(B, S, H * Dh) @ wo

    def _B_ref(x, w1, w2, w3, w4):
        B, S, D = x.shape
        h = _gelu(_layernorm(x, axis=-1) @ w1)
        c = D // 4
        g0 = jnp.pad(h[:, :, 0*c:1*c], ((0, 0), (1, 0), (0, 0)))[:, :S, :]
        g1 = jnp.pad(h[:, :, 1*c:2*c], ((0, 0), (0, 1), (0, 0)))[:, 1:, :]
        g2 = jnp.pad(h[:, :, 2*c:3*c], ((0, 0), (2, 0), (0, 0)))[:, :S, :]
        g3 = jnp.pad(h[:, :, 3*c:   ], ((0, 0), (0, 2), (0, 0)))[:, 2:, :]
        hs = jnp.concatenate([g0, g1, g2, g3], axis=-1) @ w2
        x1 = x + hs
        h2 = _gelu(_layernorm(x1, axis=-1) @ w3) @ w4
        return x1 + h2

    x = A_x
    xn = _layernorm(x, axis=-1)
    s = _A_ref(xn, A_wq, A_wk, A_wv, A_wo)
    g = _silu(_B_ref(xn, B_w1, B_w2, B_w3, B_w4))
    return x + s * g
```

```python
import jax
import jax.numpy as jnp
from jax import lax
import jax.experimental.pallas as pl
import jax.experimental.pallas.tpu as pltpu

S, D, H, DH, F = 2048, 512, 32, 16, 1792
BQ = 512
CK = 128
G = 2
XV = 128
RB = 512
PAD = 8
NC, NJ, NB = S // CK, BQ // 128, S // RB
NSTEP = (S // BQ) * H // G
LOG2E = 1.4426950408889634
f32, bf16 = jnp.float32, jnp.bfloat16


def _ln(x):
    xc = x - jnp.mean(x, axis=-1, keepdims=True)
    return xc * lax.rsqrt(jnp.mean(xc * xc, axis=-1, keepdims=True) + 1e-5)


def _gelu(x):
    c = 0.7978845608028654
    hx = 0.5 * x
    return hx + hx * jnp.tanh(x * (c + (c * 0.044715) * (x * x)))


def _dot(a, b):
    return jnp.dot(a, b, preferred_element_type=f32)


def _kernel(x_hbm, wq_hbm, wkt_hbm, wvt_hbm, wo_hbm, w1_hbm, w2_hbm, w3_hbm, w4_hbm, o_hbm,
            x_v, wq_v, wkv_v, wo_v, w1_v, w2_v, w3_v, w4_v, o_v, wt_s,
            xn_s, k_s, vt_s, h_s, qt_s, ot_s, s0, s1, m_s, kb_s, qb_s, xsem, wsem, osem):
    def xcp(r):
        rows = pl.ds(r * RB, RB)
        return pltpu.make_async_copy(x_hbm.at[rows], x_v.at[rows], xsem.at[r])

    def ocp(r):
        rows = pl.ds(r * RB, RB)
        return pltpu.make_async_copy(o_v.at[rows], o_hbm.at[rows], osem.at[r])

    wcps = [pltpu.make_async_copy(a, b, wsem.at[n]) for n, (a, b) in enumerate([
        (wq_hbm, wq_v), (wkt_hbm, wkv_v.at[0:DH]), (wvt_hbm, wkv_v.at[DH:2 * DH]), (w1_hbm, w1_v),
        (wo_hbm, wo_v), (w2_hbm, w2_v), (w3_hbm, w3_v), (w4_hbm, w4_v)])]
    for c in wcps[:3]:
        c.start()
    xcp(0).start()
    wcps[3].start()
    for r in range(1, NB):
        xcp(r).start()
    for c in wcps[4:]:
        c.start()

    h_s[0:PAD, :] = jnp.zeros((PAD, D), f32)
    h_s[S + PAD:S + 2 * PAD, :] = jnp.zeros((PAD, D), f32)
    for c in wcps[:3]:
        c.wait()
    wt_s[0:D, :] = (wq_v[...].astype(f32) * (DH ** -0.5)).T.astype(bf16)
    wt_s[D:D + 2 * DH, :] = wkv_v[...]
    wcps[3].wait()

    def abody(r, _):
        xcp(r).wait()
        r0 = pl.multiple_of(r * RB, RB)
        xn = _ln(x_v[pl.ds(r0, RB), :].astype(f32))
        xn_s[pl.ds(r0, RB), :] = xn
        t = lax.dot_general(wt_s[...], xn.astype(bf16), (((1,), (1,)), ((), ())),
                            preferred_element_type=f32)
        qt_s[:, pl.ds(r0, RB)] = (t[0:D] * LOG2E).astype(bf16)
        vt_s[:, pl.ds(r0, RB)] = t[D + DH:].astype(bf16)
        kt = jnp.concatenate([t[D:D + DH], jnp.zeros((128 - DH, RB), f32)], axis=0)
        k_s[pl.ds(r0, RB), :] = kt.T.astype(bf16)
        h_s[pl.ds(r0 + PAD, RB), :] = _gelu(_dot(_ln(xn).astype(bf16), w1_v[...]))
    lax.fori_loop(0, NB, abody, None)

    kf = k_s[0:XV, :].astype(f32)
    for d in range(DH):
        kb_s[d] = jnp.broadcast_to(kf[:, d:d + 1], (XV, 128))

    def pos(it):
        return (pl.ds(pl.multiple_of((it % H) * DH, DH), DH),
                pl.ds(pl.multiple_of((it // H) * BQ, BQ), BQ))

    def scores(qh, g, slot, c, m):
        m = list(m)
        j, nr = c % NJ, XV * NJ // NC
        rows = slice((c // NJ) * nr, (c // NJ + 1) * nr)
        cols = slice(j * 128, (j + 1) * 128)
        a = kb_s[0, rows, :] * qb_s[g, 0:1, cols]
        for d in range(1, DH):
            a = a + kb_s[d, rows, :] * qb_s[g, d:d + 1, cols]
        slot[g, rows, cols] = a
        m[j] = jnp.maximum(m[j], jnp.max(a.reshape(nr // 8, 8, 128), axis=0))
        cm = (S - XV) // NC
        lo = XV + (c * cm) // 16 * 16
        hi = XV + ((c + 1) * cm) // 16 * 16
        s = _dot(k_s[lo:hi, 0:DH], qh)
        for r in range(0, hi - lo, 16):
            slot[g, lo + r:lo + r + 16, :] = s[r:r + 16]
            for j in range(NJ):
                cols = slice(j * 128, (j + 1) * 128)
                m[j] = jnp.maximum(m[j], jnp.maximum(s[r:r + 8, cols], s[r + 8:r + 16, cols]))
        return m

    def probs(g, slot, c, m, l):
        ps = []
        for r in range(c * CK, (c + 1) * CK, 16):
            p = jnp.exp2(slot[g, r:r + 16, :] - m)
            l = l + jnp.sum(p.reshape(2, 8, BQ), axis=0)
            ps.append(p)
        return l, jnp.concatenate(ps, axis=0).astype(bf16)

    def step(j, src, dst):
        for g in range(G):
            if dst is not None:
                qh = qt_s[pos((j + 1) * G + g)]
                qb_s[g] = qh.astype(f32)
                mn = [jnp.full((8, 128), -jnp.inf, f32)] * NJ
            if src is not None:
                m = m_s[g]
                l = jnp.zeros((8, BQ), f32)
                acc = jnp.zeros((DH, BQ), f32)
            for c in range(NC):
                if src is not None:
                    l, p = probs(g, src, c, m, l)
                if dst is not None:
                    mn = scores(qh, g, dst, c, mn)
                if src is not None:
                    acc = acc + _dot(vt_s[:, c * CK:(c + 1) * CK], p)
            if src is not None:
                ot_s[pos(j * G + g)] = acc / jnp.sum(l, axis=0, keepdims=True)
            if dst is not None:
                m_s[g] = jnp.max(jnp.concatenate(mn, axis=1), axis=0, keepdims=True)

    def hbody(j, _):
        @pl.when(j % 2 == 0)
        def _():
            step(j, s0, s1)

        @pl.when(j % 2 == 1)
        def _():
            step(j, s1, s0)

    step(-1, None, s0)
    lax.fori_loop(0, NSTEP - 1, hbody, None)
    step(NSTEP - 1, (s0, s1)[(NSTEP - 1) % 2], None)

    for c in wcps[4:]:
        c.wait()

    def cbody(r, _):
        r0 = pl.multiple_of(r * RB, RB)
        sa = _dot(ot_s[:, pl.ds(r0, RB)].T.astype(bf16), wo_v[...])
        hw = h_s[pl.ds(r0, RB + 2 * PAD), :]
        hc = jnp.concatenate(
            [hw[PAD - sh:PAD - sh + RB, n * 128:(n + 1) * 128] for n, sh in enumerate((1, -1, 2, -2))],
            axis=-1)
        x1 = xn_s[pl.ds(r0, RB), :] + _dot(hc.astype(bf16), w2_v[...])
        y = _gelu(_dot(_ln(x1).astype(bf16), w3_v[...]))
        b = x1 + _dot(y.astype(bf16), w4_v[...])
        gate = b * jax.nn.sigmoid(b)
        o_v[pl.ds(r0, RB), :] = (x_v[pl.ds(r0, RB), :].astype(f32) + sa * gate).astype(bf16)
        ocp(r).start()
    lax.fori_loop(0, NB, cbody, None)
    for r in range(NB):
        ocp(r).wait()


@jax.jit
def pallas_recurrent_scan__grouped_kv_mqa__mixer_s_mlp__prompt_kernel(
    A_x, A_wq, A_wk, A_wv, A_wo, B_x, B_w1, B_w2, B_w3, B_w4,
):
    del B_x
    ins = [A_x.reshape(S, D), A_wq, A_wk.T, A_wv.T, A_wo, B_w1, B_w2, B_w3, B_w4]
    V = pltpu.VMEM
    out = pl.pallas_call(
        _kernel,
        in_specs=[pl.BlockSpec(memory_space=pl.ANY) for _ in ins],
        out_specs=pl.BlockSpec(memory_space=pl.ANY),
        out_shape=jax.ShapeDtypeStruct((S, D), bf16),
        scratch_shapes=[
            V((S, D), bf16), V((D, D), bf16), V((2 * DH, D), bf16), V((D, D), bf16),
            V((D, D), bf16), V((D, D), bf16), V((D, F), bf16), V((F, D), bf16),
            V((S, D), bf16), V((D + 2 * DH, D), bf16),
            V((S, D), f32), V((S, 128), bf16), V((DH, S), bf16), V((S + 2 * PAD, D), f32),
            V((D, S), bf16), V((D, S), f32), V((G, S, BQ), f32), V((G, S, BQ), f32),
            V((G, 1, BQ), f32), V((DH, XV, 128), f32), V((G, DH, BQ), f32),
            pltpu.SemaphoreType.DMA((NB,)), pltpu.SemaphoreType.DMA((8,)),
            pltpu.SemaphoreType.DMA((NB,))],
        compiler_params=pltpu.CompilerParams(
            flags={"XLA_TPU_EVENLY_DISTRIBUTE_CRITICAL_NODES": True},
            vmem_limit_bytes=100 * 1024 * 1024),
    )(*ins)
    return out.reshape(1, S, D)
```

```python
import jax
import jax.numpy as jnp
from jax import lax
import jax.experimental.pallas as pl
import jax.experimental.pallas.tpu as pltpu

S, D, H, DH, F = 2048, 512, 32, 16, 1792
BQ = 512
CK = 128
G, GF = 2, 4
XV, XF = 128, 288
M_SAFE = 40.0
V_SAFE = 2.0 ** -20
RB = 512
PAD = 8
NC, NJ, NB = S // CK, BQ // 128, S // RB
NITEM = (S // BQ) * H
LOG2E = 1.4426950408889634
f32, bf16 = jnp.float32, jnp.bfloat16


def _ln(x):
    xc = x - jnp.mean(x, axis=-1, keepdims=True)
    return xc * lax.rsqrt(jnp.mean(xc * xc, axis=-1, keepdims=True) + 1e-5)


def _gelu(x):
    c = 0.7978845608028654
    hx = 0.5 * x
    return hx + hx * jnp.tanh(x * (c + (c * 0.044715) * (x * x)))


def _dot(a, b):
    return jnp.dot(a, b, preferred_element_type=f32)


def _kernel(x_hbm, wq_hbm, wkt_hbm, wvt_hbm, wo_hbm, w1_hbm, w2_hbm, w3_hbm, w4_hbm, o_hbm,
            x_v, wq_v, wkv_v, wo_v, w1_v, w2_v, w3_v, w4_v, o_v, wt_s,
            xn_s, k_s, vt_s, h_s, qt_s, ot_s, s0, s1, m_s, kb_s, qb_s, k2_s, xsem, wsem, osem):
    def xcp(r):
        rows = pl.ds(r * RB, RB)
        return pltpu.make_async_copy(x_hbm.at[rows], x_v.at[rows], xsem.at[r])

    def ocp(r):
        rows = pl.ds(r * RB, RB)
        return pltpu.make_async_copy(o_v.at[rows], o_hbm.at[rows], osem.at[r])

    wcps = [pltpu.make_async_copy(a, b, wsem.at[n]) for n, (a, b) in enumerate([
        (wq_hbm, wq_v), (wkt_hbm, wkv_v.at[0:DH]), (wvt_hbm, wkv_v.at[DH:2 * DH]), (w1_hbm, w1_v),
        (wo_hbm, wo_v), (w2_hbm, w2_v), (w3_hbm, w3_v), (w4_hbm, w4_v)])]
    for c in wcps[:3]:
        c.start()
    xcp(0).start()
    wcps[3].start()
    for r in range(1, NB):
        xcp(r).start()
    for c in wcps[4:]:
        c.start()

    h_s[0:PAD, :] = jnp.zeros((PAD, D), f32)
    h_s[S + PAD:S + 2 * PAD, :] = jnp.zeros((PAD, D), f32)
    for c in wcps[:3]:
        c.wait()
    wt_s[0:D, :] = (wq_v[...].astype(f32) * (DH ** -0.5)).T.astype(bf16)
    wt_s[D:D + 2 * DH, :] = wkv_v[...]
    wcps[3].wait()

    def abody(r, carry):
        xcp(r).wait()
        r0 = pl.multiple_of(r * RB, RB)
        xn = _ln(x_v[pl.ds(r0, RB), :].astype(f32))
        xn_s[pl.ds(r0, RB), :] = xn
        t = lax.dot_general(wt_s[...], xn.astype(bf16), (((1,), (1,)), ((), ())),
                            preferred_element_type=f32)
        q = t[0:D] * LOG2E
        qt_s[:, pl.ds(r0, RB)] = q.astype(bf16)
        vt_s[:, pl.ds(r0, RB)] = t[D + DH:].astype(bf16)
        kt = jnp.concatenate([t[D:D + DH], jnp.zeros((128 - DH, RB), f32)], axis=0)
        k_s[pl.ds(r0, RB), :] = kt.T.astype(bf16)
        h_s[pl.ds(r0 + PAD, RB), :] = _gelu(_dot(_ln(xn).astype(bf16), w1_v[...]))
        q2, k2, va = carry
        qq = (q * q).reshape(H, 2, 8, RB)
        q2 = jnp.maximum(q2, jnp.max(jnp.sum(qq[:, 0] + qq[:, 1], axis=1, keepdims=True), axis=0))
        k2 = jnp.maximum(k2, jnp.sum(t[D:D + DH] * t[D:D + DH], axis=0, keepdims=True))
        return q2, k2, jnp.maximum(va, jnp.abs(t[D + DH:]))
    z = jnp.zeros((1, RB), f32)
    q2, k2, va = lax.fori_loop(0, NB, abody, (z, z, jnp.zeros((DH, RB), f32)))
    bound = jnp.sqrt(jnp.max(q2, axis=1, keepdims=True) * jnp.max(k2, axis=1, keepdims=True)) * 1.02
    bound = bound.astype(bf16).astype(f32)
    vmin = jnp.min(jnp.max(va, axis=1, keepdims=True), axis=0, keepdims=True)
    safe = jnp.max(jnp.where((bound <= M_SAFE) & (vmin >= V_SAFE), 1, 0)) == 1

    kf = k_s[0:XF, :].astype(f32)
    for d in range(DH):
        kb_s[d] = jnp.broadcast_to(kf[:, d:d + 1], (XF, 128))

    def pos(it):
        return (pl.ds(pl.multiple_of((it % H) * DH, DH), DH),
                pl.ds(pl.multiple_of((it // H) * BQ, BQ), BQ))

    def scores(qh, g, slot, c, m):
        m = list(m)
        j, nr = c % NJ, XV * NJ // NC
        rows = slice((c // NJ) * nr, (c // NJ + 1) * nr)
        cols = slice(j * 128, (j + 1) * 128)
        a = kb_s[0, rows, :] * qb_s[g, 0:1, cols]
        for d in range(1, DH):
            a = a + kb_s[d, rows, :] * qb_s[g, d:d + 1, cols]
        slot[g, rows, cols] = a
        m[j] = jnp.maximum(m[j], jnp.max(a.reshape(nr // 8, 8, 128), axis=0))
        cm = (S - XV) // NC
        lo = XV + (c * cm) // 16 * 16
        hi = XV + ((c + 1) * cm) // 16 * 16
        s = _dot(k_s[lo:hi, 0:DH], qh)
        for r in range(0, hi - lo, 16):
            slot[g, lo + r:lo + r + 16, :] = s[r:r + 16]
            for j in range(NJ):
                cols = slice(j * 128, (j + 1) * 128)
                m[j] = jnp.maximum(m[j], jnp.maximum(s[r:r + 8, cols], s[r + 8:r + 16, cols]))
        return m

    def probs(g, slot, c, m, l):
        ps = []
        for r in range(c * CK, (c + 1) * CK, 16):
            p = jnp.exp2(slot[g, r:r + 16, :] - m)
            l = l + jnp.sum(p.reshape(2, 8, BQ), axis=0)
            ps.append(p)
        return l, jnp.concatenate(ps, axis=0).astype(bf16)

    def step(j, src, dst):
        for g in range(G):
            if dst is not None:
                qh = qt_s[pos((j + 1) * G + g)]
                qb_s[g] = qh.astype(f32)
                mn = [jnp.full((8, 128), -jnp.inf, f32)] * NJ
            if src is not None:
                m = m_s[g]
                l = jnp.zeros((8, BQ), f32)
                acc = jnp.zeros((DH, BQ), f32)
            for c in range(NC):
                if src is not None:
                    l, p = probs(g, src, c, m, l)
                if dst is not None:
                    mn = scores(qh, g, dst, c, mn)
                if src is not None:
                    acc = acc + _dot(vt_s[:, c * CK:(c + 1) * CK], p)
            if src is not None:
                ot_s[pos(j * G + g)] = acc / jnp.sum(l, axis=0, keepdims=True)
            if dst is not None:
                m_s[g] = jnp.max(jnp.concatenate(mn, axis=1), axis=0, keepdims=True)

    def emit(slot, g, r, j, s16, l):
        p = jnp.exp2(s16)
        slot[g, r:r + 16, j * 128:(j + 1) * 128] = p
        l[j] = l[j] + (p[0:8] + p[8:16])

    def fstep(j, src, dst):
        ntask, ngroup = XF // 16 * NJ, (S - XF) // 16
        for g in range(GF):
            if dst is not None:
                qh = qt_s[pos((j + 1) * GF + g)]
                qb_s[g] = qh.astype(f32)
                qa = jnp.concatenate([qh, jnp.ones((DH, BQ), bf16)], axis=0)
                l = [jnp.zeros((8, 128), f32)] * NJ
            if src is not None:
                acc = jnp.zeros((DH, BQ), f32)
            task = 0
            for c in range(NC):
                if dst is not None:
                    g0, g1 = c * ngroup // NC, (c + 1) * ngroup // NC
                    kc = pltpu.bitcast(k2_s[XF // 2 + 8 * g0:XF // 2 + 8 * g1, :], bf16)
                    s = _dot(kc[:, 0:2 * DH], qa)
                    for u in range(g0, g1):
                        while task < (u + 1) * ntask // ngroup:
                            n, r = task % NJ, (task // NJ) * 16
                            a = -bound
                            for d in range(DH):
                                a = a + kb_s[d, r:r + 16, :] * qb_s[g, d:d + 1, n * 128:(n + 1) * 128]
                            emit(dst, g, r, n, a, l)
                            task += 1
                        for n in range(NJ):
                            r = (u - g0) * 16
                            emit(dst, g, XF + 16 * u, n, s[r:r + 16, n * 128:(n + 1) * 128], l)
                if src is not None:
                    keys = slice(c * CK, (c + 1) * CK)
                    acc = acc + _dot(vt_s[:, keys], src[g, keys, :].astype(bf16))
            if src is not None:
                ot_s[pos(j * GF + g)] = acc / m_s[g]
            if dst is not None:
                m_s[g] = jnp.sum(jnp.concatenate(l, axis=1), axis=0, keepdims=True)

    def pipeline(fn, nstep):
        def body(j, _):
            @pl.when(j % 2 == 0)
            def _():
                fn(j, s0, s1)

            @pl.when(j % 2 == 1)
            def _():
                fn(j, s1, s0)
        fn(-1, None, s0)
        lax.fori_loop(0, nstep - 1, body, None)
        fn(nstep - 1, (s0, s1)[(nstep - 1) % 2], None)

    @pl.when(safe)
    def _():
        lane = lax.broadcasted_iota(jnp.int32, (S, 128), 1)
        ka = jnp.where(lane == DH, -bound, k_s[...].astype(f32))
        k2_s[...] = pltpu.bitcast(ka.astype(bf16), jnp.uint32)
        pipeline(fstep, NITEM // GF)

    @pl.when(jnp.logical_not(safe))
    def _():
        pipeline(step, NITEM // G)

    for c in wcps[4:]:
        c.wait()

    def cbody(r, _):
        r0 = pl.multiple_of(r * RB, RB)
        sa = _dot(ot_s[:, pl.ds(r0, RB)].T.astype(bf16), wo_v[...])
        hw = h_s[pl.ds(r0, RB + 2 * PAD), :]
        hc = jnp.concatenate(
            [hw[PAD - sh:PAD - sh + RB, n * 128:(n + 1) * 128] for n, sh in enumerate((1, -1, 2, -2))],
            axis=-1)
        x1 = xn_s[pl.ds(r0, RB), :] + _dot(hc.astype(bf16), w2_v[...])
        y = _gelu(_dot(_ln(x1).astype(bf16), w3_v[...]))
        b = x1 + _dot(y.astype(bf16), w4_v[...])
        gate = b * jax.nn.sigmoid(b)
        o_v[pl.ds(r0, RB), :] = (x_v[pl.ds(r0, RB), :].astype(f32) + sa * gate).astype(bf16)
        ocp(r).start()
    lax.fori_loop(0, NB, cbody, None)
    for r in range(NB):
        ocp(r).wait()


@jax.jit
def pallas_recurrent_scan__grouped_kv_mqa__mixer_s_mlp__prompt_kernel(
    A_x, A_wq, A_wk, A_wv, A_wo, B_x, B_w1, B_w2, B_w3, B_w4,
):
    del B_x
    ins = [A_x.reshape(S, D), A_wq, A_wk.T, A_wv.T, A_wo, B_w1, B_w2, B_w3, B_w4]
    V = pltpu.VMEM
    out = pl.pallas_call(
        _kernel,
        in_specs=[pl.BlockSpec(memory_space=pl.ANY) for _ in ins],
        out_specs=pl.BlockSpec(memory_space=pl.ANY),
        out_shape=jax.ShapeDtypeStruct((S, D), bf16),
        scratch_shapes=[
            V((S, D), bf16), V((D, D), bf16), V((2 * DH, D), bf16), V((D, D), bf16),
            V((D, D), bf16), V((D, D), bf16), V((D, F), bf16), V((F, D), bf16),
            V((S, D), bf16), V((D + 2 * DH, D), bf16),
            V((S, D), f32), V((S, 128), bf16), V((DH, S), bf16), V((S + 2 * PAD, D), f32),
            V((D, S), bf16), V((D, S), f32), V((GF, S, BQ), f32), V((GF, S, BQ), f32),
            V((GF, 1, BQ), f32), V((DH, XF, 128), f32), V((GF, DH, BQ), f32),
            V((S // 2, 128), jnp.uint32),
            pltpu.SemaphoreType.DMA((NB,)), pltpu.SemaphoreType.DMA((8,)),
            pltpu.SemaphoreType.DMA((NB,))],
        compiler_params=pltpu.CompilerParams(
            flags={"XLA_TPU_EVENLY_DISTRIBUTE_CRITICAL_NODES": True},
            vmem_limit_bytes=100 * 1024 * 1024),
    )(*ins)
    return out.reshape(1, S, D)
```

```python
import jax
import jax.numpy as jnp
from jax import lax
import jax.experimental.pallas as pl
import jax.experimental.pallas.tpu as pltpu

S, D, H, DH, F = 2048, 512, 32, 16, 1792
BQ = 512
CK = 128
G, GF = 2, 4
XV, XF = 128, 288
M_SAFE = 40.0
V_SAFE = 2.0 ** -20
RB = 512
PAD = 8
NC, NJ, NB = S // CK, BQ // 128, S // RB
NITEM = (S // BQ) * H
LOG2E = 1.4426950408889634
f32, bf16 = jnp.float32, jnp.bfloat16


def _ln(x):
    xc = x - jnp.mean(x, axis=-1, keepdims=True)
    return xc * lax.rsqrt(jnp.mean(xc * xc, axis=-1, keepdims=True) + 1e-5)


def _gelu(x):
    c = 0.7978845608028654
    hx = 0.5 * x
    return hx + hx * jnp.tanh(x * (c + (c * 0.044715) * (x * x)))


def _dot(a, b):
    return jnp.dot(a, b, preferred_element_type=f32)


def _kernel(x_hbm, wq_hbm, wkt_hbm, wvt_hbm, wo_hbm, w1_hbm, w2_hbm, w3_hbm, w4_hbm, o_hbm,
            x_v, wq_v, wkv_v, wo_v, w1_v, w2_v, w3_v, w4_v, o_v, wt_s,
            xn_s, k_s, vt_s, h_s, qt_s, ot_s, s0, s1, m_s, kb_s, qb_s, k2_s, xsem, wsem, osem):
    def xcp(r):
        rows = pl.ds(r * RB, RB)
        return pltpu.make_async_copy(x_hbm.at[rows], x_v.at[rows], xsem.at[r])

    def ocp(r):
        rows = pl.ds(r * RB, RB)
        return pltpu.make_async_copy(o_v.at[rows], o_hbm.at[rows], osem.at[r])

    wcps = [pltpu.make_async_copy(a, b, wsem.at[n]) for n, (a, b) in enumerate([
        (wq_hbm, wq_v), (wkt_hbm, wkv_v.at[0:DH]), (wvt_hbm, wkv_v.at[DH:2 * DH]), (w1_hbm, w1_v),
        (wo_hbm, wo_v), (w2_hbm, w2_v), (w3_hbm, w3_v), (w4_hbm, w4_v)])]
    for c in wcps[:3]:
        c.start()
    xcp(0).start()
    wcps[3].start()
    for r in range(1, NB):
        xcp(r).start()
    for c in wcps[4:]:
        c.start()

    h_s[0:PAD, :] = jnp.zeros((PAD, D), f32)
    h_s[S + PAD:S + 2 * PAD, :] = jnp.zeros((PAD, D), f32)
    for c in wcps[:3]:
        c.wait()
    wt_s[0:D, :] = (wq_v[...].astype(f32) * (DH ** -0.5)).T.astype(bf16)
    wt_s[D:D + 2 * DH, :] = wkv_v[...]
    wcps[3].wait()

    def abody(r, carry):
        xcp(r).wait()
        r0 = pl.multiple_of(r * RB, RB)
        xn = _ln(x_v[pl.ds(r0, RB), :].astype(f32))
        xn_s[pl.ds(r0, RB), :] = xn
        t = lax.dot_general(wt_s[...], xn.astype(bf16), (((1,), (1,)), ((), ())),
                            preferred_element_type=f32)
        q = t[0:D] * LOG2E
        qt_s[:, pl.ds(r0, RB)] = q.astype(bf16)
        vt_s[:, pl.ds(r0, RB)] = t[D + DH:].astype(bf16)
        kt = jnp.concatenate([t[D:D + DH], jnp.zeros((128 - DH, RB), f32)], axis=0)
        k_s[pl.ds(r0, RB), :] = kt.T.astype(bf16)
        h_s[pl.ds(r0 + PAD, RB), :] = _gelu(_dot(_ln(xn).astype(bf16), w1_v[...]))
        q2, k2, va = carry
        qq = (q * q).reshape(H, 2, 8, RB)
        q2 = jnp.maximum(q2, jnp.max(jnp.sum(qq[:, 0] + qq[:, 1], axis=1, keepdims=True), axis=0))
        k2 = jnp.maximum(k2, jnp.sum(t[D:D + DH] * t[D:D + DH], axis=0, keepdims=True))
        return q2, k2, jnp.maximum(va, jnp.abs(t[D + DH:]))
    z = jnp.zeros((1, RB), f32)
    q2, k2, va = lax.fori_loop(0, NB, abody, (z, z, jnp.zeros((DH, RB), f32)))
    bound = jnp.sqrt(jnp.max(q2, axis=1, keepdims=True) * jnp.max(k2, axis=1, keepdims=True)) * 1.02
    bound = bound.astype(bf16).astype(f32)
    vmin = jnp.min(jnp.max(va, axis=1, keepdims=True), axis=0, keepdims=True)
    safe = jnp.max(jnp.where((bound <= M_SAFE) & (vmin >= V_SAFE), 1, 0)) == 1

    kf = k_s[0:XF, :].astype(f32)
    for d in range(DH):
        kb_s[d] = jnp.broadcast_to(kf[:, d:d + 1], (XF, 128))

    def pos(it):
        return (pl.ds(pl.multiple_of((it % H) * DH, DH), DH),
                pl.ds(pl.multiple_of((it // H) * BQ, BQ), BQ))

    def scores(qh, g, slot, c, m):
        m = list(m)
        j, nr = c % NJ, XV * NJ // NC
        rows = slice((c // NJ) * nr, (c // NJ + 1) * nr)
        cols = slice(j * 128, (j + 1) * 128)
        a = kb_s[0, rows, :] * qb_s[g, 0:1, cols]
        for d in range(1, DH):
            a = a + kb_s[d, rows, :] * qb_s[g, d:d + 1, cols]
        slot[g, rows, cols] = a
        m[j] = jnp.maximum(m[j], jnp.max(a.reshape(nr // 8, 8, 128), axis=0))
        cm = (S - XV) // NC
        lo = XV + (c * cm) // 16 * 16
        hi = XV + ((c + 1) * cm) // 16 * 16
        s = _dot(k_s[lo:hi, 0:DH], qh)
        for r in range(0, hi - lo, 16):
            slot[g, lo + r:lo + r + 16, :] = s[r:r + 16]
            for j in range(NJ):
                cols = slice(j * 128, (j + 1) * 128)
                m[j] = jnp.maximum(m[j], jnp.maximum(s[r:r + 8, cols], s[r + 8:r + 16, cols]))
        return m

    def probs(g, slot, c, m, l):
        ps = []
        for r in range(c * CK, (c + 1) * CK, 16):
            p = jnp.exp2(slot[g, r:r + 16, :] - m)
            l = l + jnp.sum(p.reshape(2, 8, BQ), axis=0)
            ps.append(p)
        return l, jnp.concatenate(ps, axis=0).astype(bf16)

    def step(j, src, dst):
        for g in range(G):
            if dst is not None:
                qh = qt_s[pos((j + 1) * G + g)]
                qb_s[g] = qh.astype(f32)
                mn = [jnp.full((8, 128), -jnp.inf, f32)] * NJ
            if src is not None:
                m = m_s[g]
                l = jnp.zeros((8, BQ), f32)
                acc = jnp.zeros((DH, BQ), f32)
            for c in range(NC):
                if src is not None:
                    l, p = probs(g, src, c, m, l)
                if dst is not None:
                    mn = scores(qh, g, dst, c, mn)
                if src is not None:
                    acc = acc + _dot(vt_s[:, c * CK:(c + 1) * CK], p)
            if src is not None:
                ot_s[pos(j * G + g)] = acc / jnp.sum(l, axis=0, keepdims=True)
            if dst is not None:
                m_s[g] = jnp.max(jnp.concatenate(mn, axis=1), axis=0, keepdims=True)

    def emit(slot, g, r, j, s16, l):
        p = jnp.exp2(s16)
        slot[g, r:r + 16, j * 128:(j + 1) * 128] = p
        l[j] = l[j] + (p[0:8] + p[8:16])

    def fstep(j, src, dst):
        xf = XF if src is not None else XF - 64
        ntask, ngroup = xf // 16 * NJ, (S - xf) // 16
        for g in range(GF):
            if dst is not None:
                qh = qt_s[pos((j + 1) * GF + g)]
                qb_s[g] = qh.astype(f32)
                qa = jnp.concatenate([qh, jnp.ones((DH, BQ), bf16)], axis=0)
                l = [jnp.zeros((8, 128), f32)] * NJ
            if src is not None:
                acc = jnp.zeros((DH, BQ), f32)
            task = 0
            for c in range(NC):
                if dst is not None:
                    g0, g1 = c * ngroup // NC, (c + 1) * ngroup // NC
                    kc = pltpu.bitcast(k2_s[xf // 2 + 8 * g0:xf // 2 + 8 * g1, :], bf16)
                    s = _dot(kc[:, 0:2 * DH], qa)
                    for u in range(g0, g1):
                        while task < (u + 1) * ntask // ngroup:
                            n, r = task % NJ, (task // NJ) * 16
                            a = -bound
                            for d in range(DH):
                                a = a + kb_s[d, r:r + 16, :] * qb_s[g, d:d + 1, n * 128:(n + 1) * 128]
                            emit(dst, g, r, n, a, l)
                            task += 1
                        for n in range(NJ):
                            r = (u - g0) * 16
                            emit(dst, g, xf + 16 * u, n, s[r:r + 16, n * 128:(n + 1) * 128], l)
                if src is not None:
                    keys = slice(c * CK, (c + 1) * CK)
                    acc = acc + _dot(vt_s[:, keys], src[g, keys, :].astype(bf16))
            if src is not None:
                ot_s[pos(j * GF + g)] = acc / m_s[g]
            if dst is not None:
                m_s[g] = jnp.sum(jnp.concatenate(l, axis=1), axis=0, keepdims=True)

    def pipeline(fn, nstep):
        def body(j, _):
            @pl.when(j % 2 == 0)
            def _():
                fn(j, s0, s1)

            @pl.when(j % 2 == 1)
            def _():
                fn(j, s1, s0)
        fn(-1, None, s0)
        lax.fori_loop(0, nstep - 1, body, None)
        fn(nstep - 1, (s0, s1)[(nstep - 1) % 2], None)

    @pl.when(safe)
    def _():
        lane = lax.broadcasted_iota(jnp.int32, (S, 128), 1)
        ka = jnp.where(lane == DH, -bound, k_s[...].astype(f32))
        k2_s[...] = pltpu.bitcast(ka.astype(bf16), jnp.uint32)
        pipeline(fstep, NITEM // GF)

    @pl.when(jnp.logical_not(safe))
    def _():
        pipeline(step, NITEM // G)

    for c in wcps[4:]:
        c.wait()

    def cbody(r, _):
        r0 = pl.multiple_of(r * RB, RB)
        sa = _dot(ot_s[:, pl.ds(r0, RB)].T.astype(bf16), wo_v[...])
        hw = h_s[pl.ds(r0, RB + 2 * PAD), :]
        hc = jnp.concatenate(
            [hw[PAD - sh:PAD - sh + RB, n * 128:(n + 1) * 128] for n, sh in enumerate((1, -1, 2, -2))],
            axis=-1)
        x1 = xn_s[pl.ds(r0, RB), :] + _dot(hc.astype(bf16), w2_v[...])
        y = _gelu(_dot(_ln(x1).astype(bf16), w3_v[...]))
        b = x1 + _dot(y.astype(bf16), w4_v[...])
        gate = b * jax.nn.sigmoid(b)
        o_v[pl.ds(r0, RB), :] = (x_v[pl.ds(r0, RB), :].astype(f32) + sa * gate).astype(bf16)
        ocp(r).start()
    lax.fori_loop(0, NB, cbody, None)
    for r in range(NB):
        ocp(r).wait()


@jax.jit
def pallas_recurrent_scan__grouped_kv_mqa__mixer_s_mlp__prompt_kernel(
    A_x, A_wq, A_wk, A_wv, A_wo, B_x, B_w1, B_w2, B_w3, B_w4,
):
    del B_x
    ins = [A_x.reshape(S, D), A_wq, A_wk.T, A_wv.T, A_wo, B_w1, B_w2, B_w3, B_w4]
    V = pltpu.VMEM
    out = pl.pallas_call(
        _kernel,
        in_specs=[pl.BlockSpec(memory_space=pl.ANY) for _ in ins],
        out_specs=pl.BlockSpec(memory_space=pl.ANY),
        out_shape=jax.ShapeDtypeStruct((S, D), bf16),
        scratch_shapes=[
            V((S, D), bf16), V((D, D), bf16), V((2 * DH, D), bf16), V((D, D), bf16),
            V((D, D), bf16), V((D, D), bf16), V((D, F), bf16), V((F, D), bf16),
            V((S, D), bf16), V((D + 2 * DH, D), bf16),
            V((S, D), f32), V((S, 128), bf16), V((DH, S), bf16), V((S + 2 * PAD, D), f32),
            V((D, S), bf16), V((D, S), f32), V((GF, S, BQ), f32), V((GF, S, BQ), f32),
            V((GF, 1, BQ), f32), V((DH, XF, 128), f32), V((GF, DH, BQ), f32),
            V((S // 2, 128), jnp.uint32),
            pltpu.SemaphoreType.DMA((NB,)), pltpu.SemaphoreType.DMA((8,)),
            pltpu.SemaphoreType.DMA((NB,))],
        compiler_params=pltpu.CompilerParams(
            flags={"XLA_TPU_EVENLY_DISTRIBUTE_CRITICAL_NODES": True},
            vmem_limit_bytes=100 * 1024 * 1024),
    )(*ins)
    return out.reshape(1, S, D)
```

```python
import jax
import jax.numpy as jnp
from jax import lax
import jax.experimental.pallas as pl
import jax.experimental.pallas.tpu as pltpu

S, D, H, DH, F = 2048, 512, 32, 16, 1792
BQ = 512
CK = 128
G, GF = 2, 4
XV, XF = 128, 320
M_SAFE = 40.0
V_SAFE = 2.0 ** -20
RB = 512
PAD = 8
NC, NJ, NB = S // CK, BQ // 128, S // RB
NITEM = (S // BQ) * H
LOG2E = 1.4426950408889634
f32, bf16 = jnp.float32, jnp.bfloat16


def _ln(x):
    xc = x - jnp.mean(x, axis=-1, keepdims=True)
    return xc * lax.rsqrt(jnp.mean(xc * xc, axis=-1, keepdims=True) + 1e-5)


def _gelu(x):
    c = 0.7978845608028654
    hx = 0.5 * x
    return hx + hx * jnp.tanh(x * (c + (c * 0.044715) * (x * x)))


def _dot(a, b):
    return jnp.dot(a, b, preferred_element_type=f32)


def _kernel(x_hbm, wq_hbm, wkt_hbm, wvt_hbm, wo_hbm, w1_hbm, w2_hbm, w3_hbm, w4_hbm, o_hbm,
            x_v, wq_v, wkv_v, wo_v, w1_v, w2_v, w3_v, w4_v, o_v, wt_s,
            xn_s, k_s, vt_s, h_s, qt_s, ot_s, s0, s1, m_s, kb_s, qb_s, k2_s, vf_s,
            xsem, wsem, osem):
    def xcp(r):
        rows = pl.ds(r * RB, RB)
        return pltpu.make_async_copy(x_hbm.at[rows], x_v.at[rows], xsem.at[r])

    def ocp(r):
        rows = pl.ds(r * RB, RB)
        return pltpu.make_async_copy(o_v.at[rows], o_hbm.at[rows], osem.at[r])

    wcps = [pltpu.make_async_copy(a, b, wsem.at[n]) for n, (a, b) in enumerate([
        (wq_hbm, wq_v), (wkt_hbm, wkv_v.at[0:DH]), (wvt_hbm, wkv_v.at[DH:2 * DH]), (w1_hbm, w1_v),
        (wo_hbm, wo_v), (w2_hbm, w2_v), (w3_hbm, w3_v), (w4_hbm, w4_v)])]
    for c in wcps[:3]:
        c.start()
    xcp(0).start()
    wcps[3].start()
    for r in range(1, NB):
        xcp(r).start()
    for c in wcps[4:]:
        c.start()

    h_s[0:PAD, :] = jnp.zeros((PAD, D), f32)
    h_s[S + PAD:S + 2 * PAD, :] = jnp.zeros((PAD, D), f32)
    for c in wcps[:3]:
        c.wait()
    wt_s[0:D, :] = (wq_v[...].astype(f32) * (DH ** -0.5)).T.astype(bf16)
    wt_s[D:D + 2 * DH, :] = wkv_v[...]
    wcps[3].wait()

    def abody(r, carry):
        xcp(r).wait()
        r0 = pl.multiple_of(r * RB, RB)
        xn = _ln(x_v[pl.ds(r0, RB), :].astype(f32))
        xn_s[pl.ds(r0, RB), :] = xn
        t = lax.dot_general(wt_s[...], xn.astype(bf16), (((1,), (1,)), ((), ())),
                            preferred_element_type=f32)
        q = t[0:D] * LOG2E
        qt_s[:, pl.ds(r0, RB)] = q.astype(bf16)
        vt_s[:, pl.ds(r0, RB)] = t[D + DH:].astype(bf16)
        kt = jnp.concatenate([t[D:D + DH], jnp.zeros((128 - DH, RB), f32)], axis=0)
        k_s[pl.ds(r0, RB), :] = kt.T.astype(bf16)
        h_s[pl.ds(r0 + PAD, RB), :] = _gelu(_dot(_ln(xn).astype(bf16), w1_v[...]))
        q2, k2, va = carry
        qq = (q * q).reshape(H, 2, 8, RB)
        q2 = jnp.maximum(q2, jnp.max(jnp.sum(qq[:, 0] + qq[:, 1], axis=1, keepdims=True), axis=0))
        k2 = jnp.maximum(k2, jnp.sum(t[D:D + DH] * t[D:D + DH], axis=0, keepdims=True))
        return q2, k2, jnp.maximum(va, jnp.abs(t[D + DH:]))
    z = jnp.zeros((1, RB), f32)
    q2, k2, va = lax.fori_loop(0, NB, abody, (z, z, jnp.zeros((DH, RB), f32)))
    bound = jnp.sqrt(jnp.max(q2, axis=1, keepdims=True) * jnp.max(k2, axis=1, keepdims=True)) * 1.02
    bound = bound.astype(bf16).astype(f32)
    vmin = jnp.min(jnp.max(va, axis=1, keepdims=True), axis=0, keepdims=True)
    safe = jnp.max(jnp.where((bound <= M_SAFE) & (vmin >= V_SAFE), 1, 0)) == 1

    kf = k_s[0:XF, :].astype(f32)
    for d in range(DH):
        kb_s[d] = jnp.broadcast_to(kf[:, d:d + 1], (XF, 128))

    def pos(it):
        return (pl.ds(pl.multiple_of((it % H) * DH, DH), DH),
                pl.ds(pl.multiple_of((it // H) * BQ, BQ), BQ))

    def scores(qh, g, slot, c, m):
        m = list(m)
        j, nr = c % NJ, XV * NJ // NC
        rows = slice((c // NJ) * nr, (c // NJ + 1) * nr)
        cols = slice(j * 128, (j + 1) * 128)
        a = kb_s[0, rows, :] * qb_s[g, 0:1, cols]
        for d in range(1, DH):
            a = a + kb_s[d, rows, :] * qb_s[g, d:d + 1, cols]
        slot[g, rows, cols] = a
        m[j] = jnp.maximum(m[j], jnp.max(a.reshape(nr // 8, 8, 128), axis=0))
        cm = (S - XV) // NC
        lo = XV + (c * cm) // 16 * 16
        hi = XV + ((c + 1) * cm) // 16 * 16
        s = _dot(k_s[lo:hi, 0:DH], qh)
        for r in range(0, hi - lo, 16):
            slot[g, lo + r:lo + r + 16, :] = s[r:r + 16]
            for j in range(NJ):
                cols = slice(j * 128, (j + 1) * 128)
                m[j] = jnp.maximum(m[j], jnp.maximum(s[r:r + 8, cols], s[r + 8:r + 16, cols]))
        return m

    def probs(g, slot, c, m, l):
        ps = []
        for r in range(c * CK, (c + 1) * CK, 16):
            p = jnp.exp2(slot[g, r:r + 16, :] - m)
            l = l + jnp.sum(p.reshape(2, 8, BQ), axis=0)
            ps.append(p)
        return l, jnp.concatenate(ps, axis=0).astype(bf16)

    def step(j, src, dst):
        for g in range(G):
            if dst is not None:
                qh = qt_s[pos((j + 1) * G + g)]
                qb_s[g] = qh.astype(f32)
                mn = [jnp.full((8, 128), -jnp.inf, f32)] * NJ
            if src is not None:
                m = m_s[g]
                l = jnp.zeros((8, BQ), f32)
                acc = jnp.zeros((DH, BQ), f32)
            for c in range(NC):
                if src is not None:
                    l, p = probs(g, src, c, m, l)
                if dst is not None:
                    mn = scores(qh, g, dst, c, mn)
                if src is not None:
                    acc = acc + _dot(vt_s[:, c * CK:(c + 1) * CK], p)
            if src is not None:
                ot_s[pos(j * G + g)] = acc / jnp.sum(l, axis=0, keepdims=True)
            if dst is not None:
                m_s[g] = jnp.max(jnp.concatenate(mn, axis=1), axis=0, keepdims=True)

    def emit(slot, g, r, j, s16, l):
        p = jnp.exp2(s16)
        slot[g, r:r + 16, j * 128:(j + 1) * 128] = p
        l[j] = l[j] + (p[0:8] + p[8:16])

    def fstep(j, src, dst):
        xf = XF if src is not None else XF - 80
        ntask, ngroup = xf // 16 * NJ, (S - xf) // 16
        for g in range(GF):
            if dst is not None:
                qh = qt_s[pos((j + 1) * GF + g)]
                qb_s[g] = qh.astype(f32)
                qa = jnp.concatenate([qh, jnp.ones((DH, BQ), bf16)], axis=0)
                l = [jnp.zeros((8, 128), f32)] * NJ
            if src is not None:
                acc = jnp.zeros((DH, BQ), f32)
            task = 0
            for c in range(NC):
                if dst is not None:
                    g0, g1 = c * ngroup // NC, (c + 1) * ngroup // NC
                    kc = pltpu.bitcast(k2_s[xf // 2 + 8 * g0:xf // 2 + 8 * g1, :], bf16)
                    s = _dot(kc[:, 0:2 * DH], qa)
                    for u in range(g0, g1):
                        while task < (u + 1) * ntask // ngroup:
                            n, r = task % NJ, (task // NJ) * 16
                            a = -bound
                            for d in range(DH):
                                a = a + kb_s[d, r:r + 16, :] * qb_s[g, d:d + 1, n * 128:(n + 1) * 128]
                            emit(dst, g, r, n, a, l)
                            task += 1
                        for n in range(NJ):
                            r = (u - g0) * 16
                            emit(dst, g, xf + 16 * u, n, s[r:r + 16, n * 128:(n + 1) * 128], l)
                if src is not None:
                    keys = slice(c * CK, (c + 1) * CK)
                    acc = acc + _dot(vf_s[:, keys], src[g, keys, :])
            if src is not None:
                ot_s[pos(j * GF + g)] = acc / m_s[g]
            if dst is not None:
                m_s[g] = jnp.sum(jnp.concatenate(l, axis=1), axis=0, keepdims=True)

    def pipeline(fn, nstep):
        def body(j, _):
            @pl.when(j % 2 == 0)
            def _():
                fn(j, s0, s1)

            @pl.when(j % 2 == 1)
            def _():
                fn(j, s1, s0)
        fn(-1, None, s0)
        lax.fori_loop(0, nstep - 1, body, None)
        fn(nstep - 1, (s0, s1)[(nstep - 1) % 2], None)

    @pl.when(safe)
    def _():
        lane = lax.broadcasted_iota(jnp.int32, (S, 128), 1)
        ka = jnp.where(lane == DH, -bound, k_s[...].astype(f32))
        k2_s[...] = pltpu.bitcast(ka.astype(bf16), jnp.uint32)
        vf_s[...] = vt_s[...].astype(f32)
        pipeline(fstep, NITEM // GF)

    @pl.when(jnp.logical_not(safe))
    def _():
        pipeline(step, NITEM // G)

    for c in wcps[4:]:
        c.wait()

    def cbody(r, _):
        r0 = pl.multiple_of(r * RB, RB)
        hw = h_s[pl.ds(r0, RB + 2 * PAD), :]
        hc = jnp.concatenate(
            [hw[PAD - sh:PAD - sh + RB, n * 128:(n + 1) * 128] for n, sh in enumerate((1, -1, 2, -2))],
            axis=-1)
        x1 = xn_s[pl.ds(r0, RB), :] + _dot(hc.astype(bf16), w2_v[...])
        sa = _dot(ot_s[:, pl.ds(r0, RB)].T.astype(bf16), wo_v[...])
        y = _gelu(_dot(_ln(x1).astype(bf16), w3_v[...]))
        b = x1 + _dot(y.astype(bf16), w4_v[...])
        gate = b * jax.nn.sigmoid(b)
        o_v[pl.ds(r0, RB), :] = (x_v[pl.ds(r0, RB), :].astype(f32) + sa * gate).astype(bf16)
        ocp(r).start()
    lax.fori_loop(0, NB, cbody, None)
    for r in range(NB):
        ocp(r).wait()


@jax.jit
def pallas_recurrent_scan__grouped_kv_mqa__mixer_s_mlp__prompt_kernel(
    A_x, A_wq, A_wk, A_wv, A_wo, B_x, B_w1, B_w2, B_w3, B_w4,
):
    del B_x
    ins = [A_x.reshape(S, D), A_wq, A_wk.T, A_wv.T, A_wo, B_w1, B_w2, B_w3, B_w4]
    V = pltpu.VMEM
    out = pl.pallas_call(
        _kernel,
        in_specs=[pl.BlockSpec(memory_space=pl.ANY) for _ in ins],
        out_specs=pl.BlockSpec(memory_space=pl.ANY),
        out_shape=jax.ShapeDtypeStruct((S, D), bf16),
        scratch_shapes=[
            V((S, D), bf16), V((D, D), bf16), V((2 * DH, D), bf16), V((D, D), bf16),
            V((D, D), bf16), V((D, D), bf16), V((D, F), bf16), V((F, D), bf16),
            V((S, D), bf16), V((D + 2 * DH, D), bf16),
            V((S, D), f32), V((S, 128), bf16), V((DH, S), bf16), V((S + 2 * PAD, D), f32),
            V((D, S), bf16), V((D, S), f32), V((GF, S, BQ), f32), V((GF, S, BQ), f32),
            V((GF, 1, BQ), f32), V((DH, XF, 128), f32), V((GF, DH, BQ), f32),
            V((S // 2, 128), jnp.uint32), V((DH, S), f32),
            pltpu.SemaphoreType.DMA((NB,)), pltpu.SemaphoreType.DMA((8,)),
            pltpu.SemaphoreType.DMA((NB,))],
        compiler_params=pltpu.CompilerParams(
            flags={"XLA_TPU_EVENLY_DISTRIBUTE_CRITICAL_NODES": True},
            vmem_limit_bytes=100 * 1024 * 1024),
    )(*ins)
    return out.reshape(1, S, D)
```
